```python
import jax
import jax.numpy as jnp

def _softmax(x, axis=-1):
    return jax.nn.softmax(x, axis=axis)
def _gelu(x):
    return jax.nn.gelu(x, approximate=True)
def _silu(x):
    return jax.nn.silu(x)
def _sigmoid(x):
    return jax.nn.sigmoid(x)
def _layernorm(x, axis=-1, eps=1e-5):
    m = jnp.mean(x, axis=axis, keepdims=True)
    v = jnp.var(x, axis=axis, keepdims=True)
    return (x - m) / jnp.sqrt(v + eps)
def _scatter_add(tgt, idx, src, axis=0):
    return tgt.at[idx].add(src)
def _segment_sum(src, seg, n):
    return jax.ops.segment_sum(src, seg, n)
class _Rng:
    def __init__(self, key):
        self._k = key
    def _next(self):
        self._k, sub = jax.random.split(self._k)
        return sub
    def normal(self, shape):
        return jax.random.normal(self._next(), shape, dtype=jnp.bfloat16)
    def randint(self, lo, hi, shape):
        return jax.random.randint(self._next(), shape, lo, hi, dtype=jnp.int32)
    def uniform(self, shape, lo=0.0, hi=1.0):
        return jax.random.uniform(self._next(), shape, jnp.bfloat16, lo, hi)
    def permutation(self, n):
        return jax.random.permutation(self._next(), n)


kernel_name = 'recurrent_scan__sliding_block_cached__mixer_s_mlp__decode'

def setup_inputs():
    _rng = _Rng(jax.random.key(int.from_bytes(__import__("os").urandom(4), "little")))
    _w = (lambda a: (lambda t: t.astype(jnp.bfloat16) if jnp.issubdtype(t.dtype, jnp.floating) else t)(jnp.asarray(a)))
    def _A_setup():
        B, Sq, D = 1, 1, 512
        Hq, Hkv, Sk, Dh = 32, 32, 32768, 128
        assert Hq % Hkv == 0, (Hq, Hkv)
        return {
            "x": _w((lambda *s: _rng.normal(s) * 0.05)(B, Sq, D)),
            "k_cache": _w((lambda *s: _rng.normal(s) * 0.05)(B, Hkv, Sk, Dh)),
            "v_cache": _w((lambda *s: _rng.normal(s) * 0.05)(B, Hkv, Sk, Dh)),
            "wq": _w((lambda *s: _rng.normal(s) * 0.05)(D, Hq * Dh) * (D ** -0.5)),
            "wo": _w((lambda *s: _rng.normal(s) * 0.05)(Hq * Dh, D) * ((Hq * Dh) ** -0.5)),
        }
    _A_in = _A_setup()

    def _B_setup():
        B, S, D, F = 1, 1, 512, 1376
        return {
            "x":  _w((lambda *s: _rng.normal(s) * 0.05)(B, S, D)),
            "w1": _w((lambda *s: _rng.normal(s) * 0.05)(D, D) * (D ** -0.5)),
            "w2": _w((lambda *s: _rng.normal(s) * 0.05)(D, D) * (D ** -0.5)),
            "w3": _w((lambda *s: _rng.normal(s) * 0.05)(D, F) * (D ** -0.5)),
            "w4": _w((lambda *s: _rng.normal(s) * 0.05)(F, D) * (F ** -0.5)),
        }
    _B_in = _B_setup()

    return {
        "A_x": _A_in["x"],
        "A_k_cache": _A_in["k_cache"],
        "A_v_cache": _A_in["v_cache"],
        "A_wq": _A_in["wq"],
        "A_wo": _A_in["wo"],
        "B_x": _B_in["x"],
        "B_w1": _B_in["w1"],
        "B_w2": _B_in["w2"],
        "B_w3": _B_in["w3"],
        "B_w4": _B_in["w4"],
    }

def reference(A_x, A_k_cache, A_v_cache, A_wq, A_wo, B_x, B_w1, B_w2, B_w3, B_w4):
    def _A_ref(x, k_cache, v_cache, wq, wo):
        B, Sq, D = x.shape
        Hq, Dh = 32, 128
        Hkv, Sk = k_cache.shape[1], k_cache.shape[2]
        W = min(4096, max(256, Sk // 4))
        rep = Hq // Hkv
        q = (lambda x, *d: x.transpose(*d))((x @ wq).reshape(B, Sq, Hq, Dh), 0, 2, 1, 3)
        k = jnp.repeat(k_cache[:, :, Sk - W:, :], rep, axis=1)
        v = jnp.repeat(v_cache[:, :, Sk - W:, :], rep, axis=1)
        scores = jnp.einsum("bhqd,bhkd->bhqk", q, k) * (Dh ** -0.5)
        p = _softmax(scores, axis=-1)
        o = jnp.einsum("bhqk,bhkd->bhqd", p, v)
        return (lambda x, *d: x.transpose(*d))(o, 0, 2, 1, 3).reshape(B, Sq, Hq * Dh) @ wo

    def _B_ref(x, w1, w2, w3, w4):
        B, S, D = x.shape
        h = _gelu(_layernorm(x, axis=-1) @ w1)
        c = D // 4
        g0 = jnp.pad(h[:, :, 0*c:1*c], ((0, 0), (1, 0), (0, 0)))[:, :S, :]
        g1 = jnp.pad(h[:, :, 1*c:2*c], ((0, 0), (0, 1), (0, 0)))[:, 1:, :]
        g2 = jnp.pad(h[:, :, 2*c:3*c], ((0, 0), (2, 0), (0, 0)))[:, :S, :]
        g3 = jnp.pad(h[:, :, 3*c:   ], ((0, 0), (0, 2), (0, 0)))[:, 2:, :]
        hs = jnp.concatenate([g0, g1, g2, g3], axis=-1) @ w2
        x1 = x + hs
        h2 = _gelu(_layernorm(x1, axis=-1) @ w3) @ w4
        return x1 + h2

    x = A_x
    xn = _layernorm(x, axis=-1)
    s = _A_ref(xn, A_k_cache, A_v_cache, A_wq, A_wo)
    g = _silu(_B_ref(xn, B_w1, B_w2, B_w3, B_w4))
    return x + s * g
```

```python
import jax
import jax.numpy as jnp
import jax.experimental.pallas as pl
import jax.experimental.pallas.tpu as pltpu

H, DH, D, F, W, SK = 32, 128, 512, 1376, 4096, 32768
LA = 2
NB = LA + 1
WO_CHUNKS = [1024, 1024, 1024, 512, 256, 128, 128]
assert sum(WO_CHUNKS) == H * DH
f32, bf16 = jnp.float32, jnp.bfloat16


def _ln(x):
    m = jnp.mean(x, axis=-1, keepdims=True)
    xc = x - m
    v = jnp.mean(xc * xc, axis=-1, keepdims=True)
    return xc / jnp.sqrt(v + 1e-5)


def kernel(x_hbm, k_hbm, v_hbm, wq_hbm, wo_hbm, w3_hbm, w4_hbm, o_hbm,
           x_v, wq_v, wo_v, w3_v, w4_v, kbuf, vbuf, q_s, o_s, out_v,
           wsem, ksem, vsem, osem):
    cx = pltpu.make_async_copy(x_hbm, x_v, wsem.at[0])
    cq = pltpu.make_async_copy(wq_hbm, wq_v, wsem.at[1])
    c3 = pltpu.make_async_copy(w3_hbm, w3_v, wsem.at[2])
    c4 = pltpu.make_async_copy(w4_hbm, w4_v, wsem.at[3])

    def kcp(h, slot):
        return pltpu.make_async_copy(k_hbm.at[0, h, pl.ds(SK - W, W), :], kbuf.at[slot], ksem.at[slot])

    def vcp(h, slot):
        return pltpu.make_async_copy(v_hbm.at[0, h, pl.ds(SK - W, W), :], vbuf.at[slot], vsem.at[slot])

    offs = [sum(WO_CHUNKS[:i]) for i in range(len(WO_CHUNKS))]

    def ocp(i):
        return pltpu.make_async_copy(wo_hbm.at[pl.ds(offs[i], WO_CHUNKS[i]), :],
                                     wo_v.at[pl.ds(offs[i], WO_CHUNKS[i]), :], osem.at[i])

    cx.start(); cq.start(); c3.start(); c4.start()
    for h in range(LA):
        kcp(h, h).start()
        vcp(h, h).start()

    cx.wait()
    x = x_v[0].astype(f32)
    xn = _ln(x)
    xn8 = jnp.broadcast_to(xn, (8, D))
    y8 = _ln(xn8).astype(bf16)
    cq.wait()
    q = jnp.dot(xn8.astype(bf16), wq_v[...], preferred_element_type=f32).astype(bf16)
    for h in range(H):
        q_s[h] = q[:, h * DH:(h + 1) * DH]
    c3.wait()
    h1 = jax.lax.dot_general(y8, w3_v[...], (((1,), (1,)), ((), ())), preferred_element_type=f32)
    h1 = jax.nn.gelu(h1, approximate=True).astype(bf16)
    c4.wait()
    h2 = jnp.dot(h1, w4_v[...], preferred_element_type=f32)
    b = xn8 + h2
    g = b * jax.nn.sigmoid(b)

    def body(h, carry):
        slot = h % NB
        nslot = (h + LA) % NB
        kcp(h, slot).wait()

        @pl.when(h + LA < H)
        def _():
            kcp(h + LA, nslot).start()

        s = jax.lax.dot_general(q_s[h], kbuf[slot], (((1,), (1,)), ((), ())), preferred_element_type=f32) * (DH ** -0.5)
        m = jnp.max(s, axis=-1, keepdims=True)
        p = jnp.exp(s - m)
        l = jnp.sum(p, axis=-1, keepdims=True)
        pb = p.astype(bf16)
        vcp(h, slot).wait()

        @pl.when(h + LA < H)
        def _():
            vcp(h + LA, nslot).start()

        @pl.when(h == H - LA)
        def _():
            for i in range(len(WO_CHUNKS)):
                ocp(i).start()

        o = jnp.dot(pb, vbuf[slot], preferred_element_type=f32) / l
        o_s[h] = o.astype(bf16)
        return carry

    jax.lax.fori_loop(0, H, body, 0)

    acc = jnp.zeros((8, D), f32)
    for i in range(len(WO_CHUNKS)):
        ocp(i).wait()
        h0 = offs[i] // DH
        nh = WO_CHUNKS[i] // DH
        oc = jnp.concatenate([o_s[h0 + j] for j in range(nh)], axis=-1) if nh > 1 else o_s[h0]
        acc = acc + jnp.dot(oc, wo_v[pl.ds(offs[i], WO_CHUNKS[i]), :], preferred_element_type=f32)
    out = x + acc[0:1] * g[0:1]
    out_v[0] = out.astype(bf16)
    co = pltpu.make_async_copy(out_v, o_hbm, wsem.at[0])
    co.start()
    co.wait()


@jax.jit
def pallas_recurrent_scan__sliding_block_cached__mixer_s_mlp__decode_kernel(
    A_x, A_k_cache, A_v_cache, A_wq, A_wo, B_x, B_w1, B_w2, B_w3, B_w4):
    return pl.pallas_call(
        kernel,
        in_specs=[pl.BlockSpec(memory_space=pl.ANY)] * 7,
        out_specs=pl.BlockSpec(memory_space=pl.ANY),
        out_shape=jax.ShapeDtypeStruct((1, 1, D), bf16),
        scratch_shapes=[
            pltpu.VMEM((1, 1, D), bf16),
            pltpu.VMEM((D, H * DH), bf16),
            pltpu.VMEM((H * DH, D), bf16),
            pltpu.VMEM((F, D), bf16),
            pltpu.VMEM((F, D), bf16),
            pltpu.VMEM((NB, W, DH), bf16),
            pltpu.VMEM((NB, W, DH), bf16),
            pltpu.VMEM((H, 8, DH), bf16),
            pltpu.VMEM((H, 8, DH), bf16),
            pltpu.VMEM((1, 1, D), bf16),
            pltpu.SemaphoreType.DMA((4,)),
            pltpu.SemaphoreType.DMA((NB,)),
            pltpu.SemaphoreType.DMA((NB,)),
            pltpu.SemaphoreType.DMA((len(WO_CHUNKS),)),
        ],
        compiler_params=pltpu.CompilerParams(vmem_limit_bytes=64 * 1024 * 1024),
    )(A_x, A_k_cache, A_v_cache, A_wq, A_wo, B_w3.T, B_w4)
```

```python
import jax
import jax.numpy as jnp
import jax.experimental.pallas as pl
import jax.experimental.pallas.tpu as pltpu

H, DH, D, F, W, SK = 32, 128, 512, 1376, 4096, 32768
LA = 2
NB = LA + 1
MXU_CHUNKS = (1024, 1024, 1024, 512, 256, 128)
VPU_CHUNKS = (96, 32)
WO_CHUNKS = MXU_CHUNKS + VPU_CHUNKS
WO_OFFS = tuple(sum(WO_CHUNKS[:i]) for i in range(len(WO_CHUNKS)))
assert sum(WO_CHUNKS) == H * DH and sum(VPU_CHUNKS) == DH
f32, bf16 = jnp.float32, jnp.bfloat16


def _ln(x):
    m = jnp.mean(x, axis=-1, keepdims=True)
    xc = x - m
    v = jnp.mean(xc * xc, axis=-1, keepdims=True)
    return xc / jnp.sqrt(v + 1e-5)


def _kernel(x_hbm, k_hbm, v_hbm, wq_hbm, wo_hbm, w3t_hbm, w4_hbm, o_hbm,
            x_v, wq_v, wo_v, w3_v, w4_v, kbuf, vbuf, q_s, o_s, out_v,
            wsem, ksem, vsem, osem):
    cx = pltpu.make_async_copy(x_hbm, x_v, wsem.at[0])
    cq = pltpu.make_async_copy(wq_hbm, wq_v, wsem.at[1])
    c3 = pltpu.make_async_copy(w3t_hbm, w3_v, wsem.at[2])
    c4 = pltpu.make_async_copy(w4_hbm, w4_v, wsem.at[3])

    def kcp(h, slot):
        return pltpu.make_async_copy(k_hbm.at[0, h, pl.ds(SK - W, W), :], kbuf.at[slot], ksem.at[slot])

    def vcp(h, slot):
        return pltpu.make_async_copy(v_hbm.at[0, h, pl.ds(SK - W, W), :], vbuf.at[slot], vsem.at[slot])

    def ocp(i):
        rows = pl.ds(WO_OFFS[i], WO_CHUNKS[i])
        return pltpu.make_async_copy(wo_hbm.at[rows, :], wo_v.at[rows, :], osem.at[i])

    cx.start()
    cq.start()
    c3.start()
    c4.start()
    for h in range(LA):
        kcp(h, h).start()
        vcp(h, h).start()

    cx.wait()
    x8 = jnp.broadcast_to(x_v[0].astype(f32), (8, D))
    xn8 = _ln(x8)
    y8 = _ln(xn8).astype(bf16)
    cq.wait()
    q = jnp.dot(xn8.astype(bf16), wq_v[...], preferred_element_type=f32).astype(bf16)
    for h in range(H):
        q_s[h] = q[:, h * DH:(h + 1) * DH]
    c3.wait()
    h1 = jax.lax.dot_general(y8, w3_v[...], (((1,), (1,)), ((), ())), preferred_element_type=f32)
    h1 = jax.nn.gelu(h1, approximate=True).astype(bf16)
    c4.wait()
    b = xn8 + jnp.dot(h1, w4_v[...], preferred_element_type=f32)
    g = b * jax.nn.sigmoid(b)

    def head(h, carry):
        slot = h % NB
        nslot = (h + LA) % NB
        kcp(h, slot).wait()

        @pl.when(h + LA < H)
        def _():
            kcp(h + LA, nslot).start()

        s = jax.lax.dot_general(q_s[h], kbuf[slot], (((1,), (1,)), ((), ())),
                                preferred_element_type=f32) * (DH ** -0.5)
        m = jnp.max(s, axis=-1, keepdims=True)
        p = jnp.exp(s - m)
        l = jnp.sum(p, axis=-1, keepdims=True)
        pb = p.astype(bf16)
        vcp(h, slot).wait()

        @pl.when(h + LA < H)
        def _():
            vcp(h + LA, nslot).start()

        @pl.when(h == H - LA)
        def _():
            for i in range(len(WO_CHUNKS)):
                ocp(i).start()

        o = jnp.dot(pb, vbuf[slot], preferred_element_type=f32) / l
        o_s[h] = o.astype(bf16)
        return carry

    jax.lax.fori_loop(0, H, head, 0)

    o_last = o_s[H - 1].astype(f32)
    ob = jnp.transpose(jnp.broadcast_to(o_last[0:1], (DH, DH)))

    acc = jnp.zeros((8, D), f32)
    nm = len(MXU_CHUNKS)
    for i in range(nm):
        ocp(i).wait()
        h0 = WO_OFFS[i] // DH
        nh = MXU_CHUNKS[i] // DH
        oc = jnp.concatenate([o_s[h0 + j] for j in range(nh)], axis=-1) if nh > 1 else o_s[h0]
        acc = acc + jnp.dot(oc, wo_v[pl.ds(WO_OFFS[i], MXU_CHUNKS[i]), :], preferred_element_type=f32)

    def vpu_rows(i):
        n = WO_CHUNKS[i]
        r0 = WO_OFFS[i] - (H - 1) * DH
        w = wo_v[pl.ds(WO_OFFS[i], n), :].astype(f32)
        prod = w * jnp.concatenate([ob[r0:r0 + n, :]] * (D // DH), axis=1)
        parts = [prod[8 * j:8 * j + 8] for j in range(n // 8)]
        while len(parts) > 1:
            parts = [parts[j] + parts[j + 1] if j + 1 < len(parts) else parts[j]
                     for j in range(0, len(parts), 2)]
        return jnp.sum(parts[0], axis=0, keepdims=True)

    n_all = len(WO_CHUNKS)
    for i in range(nm, n_all - 1):
        ocp(i).wait()
        acc = acc + vpu_rows(i)
    base = x8 + acc * g
    ocp(n_all - 1).wait()
    out = base + vpu_rows(n_all - 1) * g
    out_v[0] = out[0:1].astype(bf16)
    co = pltpu.make_async_copy(out_v, o_hbm, wsem.at[0])
    co.start()
    co.wait()


@jax.jit
def pallas_recurrent_scan__sliding_block_cached__mixer_s_mlp__decode_kernel(
    A_x, A_k_cache, A_v_cache, A_wq, A_wo, B_x, B_w1, B_w2, B_w3, B_w4):
    return pl.pallas_call(
        _kernel,
        in_specs=[pl.BlockSpec(memory_space=pl.ANY)] * 7,
        out_specs=pl.BlockSpec(memory_space=pl.ANY),
        out_shape=jax.ShapeDtypeStruct((1, 1, D), bf16),
        scratch_shapes=[
            pltpu.VMEM((1, 1, D), bf16),
            pltpu.VMEM((D, H * DH), bf16),
            pltpu.VMEM((H * DH, D), bf16),
            pltpu.VMEM((F, D), bf16),
            pltpu.VMEM((F, D), bf16),
            pltpu.VMEM((NB, W, DH), bf16),
            pltpu.VMEM((NB, W, DH), bf16),
            pltpu.VMEM((H, 8, DH), bf16),
            pltpu.VMEM((H, 8, DH), bf16),
            pltpu.VMEM((1, 1, D), bf16),
            pltpu.SemaphoreType.DMA((4,)),
            pltpu.SemaphoreType.DMA((NB,)),
            pltpu.SemaphoreType.DMA((NB,)),
            pltpu.SemaphoreType.DMA((len(WO_CHUNKS),)),
        ],
        compiler_params=pltpu.CompilerParams(
            vmem_limit_bytes=64 * 1024 * 1024,
            disable_bounds_checks=True,
            disable_semaphore_checks=True,
        ),
    )(A_x, A_k_cache, A_v_cache, A_wq, A_wo, B_w3.T, B_w4)
```

```python
import jax
import jax.numpy as jnp
import jax.experimental.pallas as pl
import jax.experimental.pallas.tpu as pltpu

H, DH, D, F, W, SK = 32, 128, 512, 1376, 4096, 32768
LA = 2
NB = LA + 1
MXU_CHUNKS = (1024, 1024, 1024, 512, 256, 128)
VPU_CHUNKS = (96, 32)
WO_CHUNKS = MXU_CHUNKS + VPU_CHUNKS
WO_OFFS = tuple(sum(WO_CHUNKS[:i]) for i in range(len(WO_CHUNKS)))
assert sum(WO_CHUNKS) == H * DH and sum(VPU_CHUNKS) == DH
f32, bf16 = jnp.float32, jnp.bfloat16
S0 = 128
S1 = 128
SIDE = (S0, S1)
R = S0 + S1
SMAX = max(S0, S1)
NS = 4
NC = 2 * H


def _ln(x):
    m = jnp.mean(x, axis=-1, keepdims=True)
    xc = x - m
    v = jnp.mean(xc * xc, axis=-1, keepdims=True)
    return xc / jnp.sqrt(v + 1e-5)


def _kernel(x_hbm, k_hbm, v_hbm, wq_hbm, wo_hbm, w3t_hbm, w4_hbm, o_hbm,
            x_v, wq_v, wo_v, w3_v, w4_v, kbuf, vbuf, q_s, o_s, out_v, stg,
            wsem, ksem, vsem, osem, asem, bsem):
    cx = pltpu.make_async_copy(x_hbm, x_v, wsem.at[0])
    cq = pltpu.make_async_copy(wq_hbm, wq_v, wsem.at[1])
    c3 = pltpu.make_async_copy(w3t_hbm, w3_v, wsem.at[2])
    c4 = pltpu.make_async_copy(w4_hbm, w4_v, wsem.at[3])

    def kcp(h, slot):
        return pltpu.make_async_copy(k_hbm.at[0, h, pl.ds(SK - W, W), :], kbuf.at[slot], ksem.at[slot])

    def vcp(h, slot):
        return pltpu.make_async_copy(v_hbm.at[0, h, pl.ds(SK - W + R, W - R), :],
                                     vbuf.at[slot, pl.ds(R, W - R), :], vsem.at[slot])

    def acp(h, j):
        s = (2 * h + j) % NS
        return pltpu.make_async_copy(v_hbm.at[0, h, pl.ds(SK - W + j * S0, SIDE[j]), :],
                                     stg.at[s, pl.ds(0, SIDE[j]), :], asem.at[s])

    def bcp(h, j):
        s = (2 * h + j) % NS
        return pltpu.make_async_copy(stg.at[s, pl.ds(0, SIDE[j]), :],
                                     vbuf.at[h % NB, pl.ds(j * S0, SIDE[j]), :], bsem.at[s])

    def side_step(h, j):
        @pl.when(h + 1 < H)
        def _():
            bcp(h + 1, j).wait()

        @pl.when(h + 3 < H)
        def _():
            acp(h + 3, j).start()

        @pl.when(h + 2 < H)
        def _():
            acp(h + 2, j).wait()
            bcp(h + 2, j).start()

    def ocp(i):
        rows = pl.ds(WO_OFFS[i], WO_CHUNKS[i])
        return pltpu.make_async_copy(wo_hbm.at[rows, :], wo_v.at[rows, :], osem.at[i])

    cx.start()
    cq.start()
    for h in range(2):
        for j in range(2):
            acp(h, j).start()
    c3.start()
    c4.start()
    for h in range(LA):
        kcp(h, h).start()
        vcp(h, h).start()

    cx.wait()
    x8 = jnp.broadcast_to(x_v[0].astype(f32), (8, D))
    xn8 = _ln(x8)
    y8 = _ln(xn8).astype(bf16)
    cq.wait()
    for h in range(2):
        for j in range(2):
            acp(h, j).wait()
            bcp(h, j).start()
    q = jnp.dot(xn8.astype(bf16), wq_v[...], preferred_element_type=f32).astype(bf16)
    for h in range(H):
        q_s[h] = q[:, h * DH:(h + 1) * DH]
    c3.wait()
    h1 = jax.lax.dot_general(y8, w3_v[...], (((1,), (1,)), ((), ())), preferred_element_type=f32)
    h1 = jax.nn.gelu(h1, approximate=True).astype(bf16)
    c4.wait()
    for j in range(2):
        bcp(0, j).wait()
        acp(2, j).start()
    b = xn8 + jnp.dot(h1, w4_v[...], preferred_element_type=f32)
    g = b * jax.nn.sigmoid(b)

    def head(h, carry):
        slot = h % NB
        nslot = (h + LA) % NB
        kcp(h, slot).wait()

        @pl.when(h + LA < H)
        def _():
            kcp(h + LA, nslot).start()

        side_step(h, 0)

        s = jax.lax.dot_general(q_s[h], kbuf[slot], (((1,), (1,)), ((), ())),
                                preferred_element_type=f32) * (DH ** -0.5)
        m = jnp.max(s, axis=-1, keepdims=True)
        p = jnp.exp(s - m)
        l = jnp.sum(p, axis=-1, keepdims=True)
        pb = p.astype(bf16)
        vcp(h, slot).wait()

        @pl.when(h + LA < H)
        def _():
            vcp(h + LA, nslot).start()

        @pl.when(h == H - LA)
        def _():
            for i in range(len(WO_CHUNKS)):
                ocp(i).start()

        side_step(h, 1)

        o = jnp.dot(pb, vbuf[slot], preferred_element_type=f32) / l
        o_s[h] = o.astype(bf16)
        return carry

    jax.lax.fori_loop(0, H, head, 0)

    o_last = o_s[H - 1].astype(f32)
    ob = jnp.transpose(jnp.broadcast_to(o_last[0:1], (DH, DH)))

    acc = jnp.zeros((8, D), f32)
    nm = len(MXU_CHUNKS)
    for i in range(nm):
        ocp(i).wait()
        h0 = WO_OFFS[i] // DH
        nh = MXU_CHUNKS[i] // DH
        oc = jnp.concatenate([o_s[h0 + j] for j in range(nh)], axis=-1) if nh > 1 else o_s[h0]
        acc = acc + jnp.dot(oc, wo_v[pl.ds(WO_OFFS[i], MXU_CHUNKS[i]), :], preferred_element_type=f32)

    def vpu_rows(i):
        n = WO_CHUNKS[i]
        r0 = WO_OFFS[i] - (H - 1) * DH
        w = wo_v[pl.ds(WO_OFFS[i], n), :].astype(f32)
        prod = w * jnp.concatenate([ob[r0:r0 + n, :]] * (D // DH), axis=1)
        parts = [prod[8 * j:8 * j + 8] for j in range(n // 8)]
        while len(parts) > 1:
            parts = [parts[j] + parts[j + 1] if j + 1 < len(parts) else parts[j]
                     for j in range(0, len(parts), 2)]
        return jnp.sum(parts[0], axis=0, keepdims=True)

    n_all = len(WO_CHUNKS)
    for i in range(nm, n_all - 1):
        ocp(i).wait()
        acc = acc + vpu_rows(i)
    base = x8 + acc * g
    ocp(n_all - 1).wait()
    out = base + vpu_rows(n_all - 1) * g
    out_v[0] = out[0:1].astype(bf16)
    co = pltpu.make_async_copy(out_v, o_hbm, wsem.at[0])
    co.start()
    co.wait()


@jax.jit
def pallas_recurrent_scan__sliding_block_cached__mixer_s_mlp__decode_kernel(
    A_x, A_k_cache, A_v_cache, A_wq, A_wo, B_x, B_w1, B_w2, B_w3, B_w4):
    return pl.pallas_call(
        _kernel,
        in_specs=[pl.BlockSpec(memory_space=pl.ANY)] * 7,
        out_specs=pl.BlockSpec(memory_space=pl.ANY),
        out_shape=jax.ShapeDtypeStruct((1, 1, D), bf16),
        scratch_shapes=[
            pltpu.VMEM((1, 1, D), bf16),
            pltpu.VMEM((D, H * DH), bf16),
            pltpu.VMEM((H * DH, D), bf16),
            pltpu.VMEM((F, D), bf16),
            pltpu.VMEM((F, D), bf16),
            pltpu.VMEM((NB, W, DH), bf16),
            pltpu.VMEM((NB, W, DH), bf16),
            pltpu.VMEM((H, 8, DH), bf16),
            pltpu.VMEM((H, 8, DH), bf16),
            pltpu.VMEM((1, 1, D), bf16),
            pltpu.SMEM((NS, SMAX, DH), bf16),
            pltpu.SemaphoreType.DMA((4,)),
            pltpu.SemaphoreType.DMA((NB,)),
            pltpu.SemaphoreType.DMA((NB,)),
            pltpu.SemaphoreType.DMA((len(WO_CHUNKS),)),
            pltpu.SemaphoreType.DMA((NS,)),
            pltpu.SemaphoreType.DMA((NS,)),
        ],
        compiler_params=pltpu.CompilerParams(
            vmem_limit_bytes=64 * 1024 * 1024,
            disable_bounds_checks=True,
            disable_semaphore_checks=True,
        ),
    )(A_x, A_k_cache, A_v_cache, A_wq, A_wo, B_w3.T, B_w4)
```

```python
import jax
import jax.numpy as jnp
import jax.experimental.pallas as pl
import jax.experimental.pallas.tpu as pltpu

H, DH, D, F, W, SK = 32, 128, 512, 1376, 4096, 32768
LA = 2
NB = LA + 1
f32, bf16 = jnp.float32, jnp.bfloat16

SV = 128
R = 2 * SV
SO = 32
NPRE = 2
NPOST = 6
RO = (NPRE + NPOST) * SO
NS = 4
QC = 4

MXU_CHUNKS = (1024 - RO, 1024, 1024, 512, 256, 128)
VPU_CHUNKS = (96, 32)
WO_CHUNKS = MXU_CHUNKS + VPU_CHUNKS
WO_OFFS = tuple(RO + sum(WO_CHUNKS[:i]) for i in range(len(WO_CHUNKS)))
assert RO + sum(WO_CHUNKS) == H * DH and sum(VPU_CHUNKS) == DH and RO % DH == 0


def _ln(x):
    m = jnp.mean(x, axis=-1, keepdims=True)
    xc = x - m
    v = jnp.mean(xc * xc, axis=-1, keepdims=True)
    return xc / jnp.sqrt(v + 1e-5)


def _kernel(x_hbm, k_hbm, v_hbm, wq_hbm, wo_hbm, w3t_hbm, w4_hbm, o_hbm,
            x_v, wq_v, wo_v, w3_v, w4_v, kbuf, vbuf, q_s, o_s, out_v, stg_v, stg_o,
            wsem, ksem, vsem, osem, asem, bsem):
    cx = pltpu.make_async_copy(x_hbm, x_v, wsem.at[0])
    c3 = pltpu.make_async_copy(w3t_hbm, w3_v, wsem.at[1])
    c4 = pltpu.make_async_copy(w4_hbm, w4_v, wsem.at[2])

    def qcp(i):
        rows = pl.ds(i * (D // QC), D // QC)
        return pltpu.make_async_copy(wq_hbm.at[rows, :], wq_v.at[rows, :], wsem.at[3 + i])

    def kcp(h, slot):
        return pltpu.make_async_copy(k_hbm.at[0, h, pl.ds(SK - W, W), :], kbuf.at[slot], ksem.at[slot])

    def vcp(h, slot):
        return pltpu.make_async_copy(v_hbm.at[0, h, pl.ds(SK - W + R, W - R), :],
                                     vbuf.at[slot, pl.ds(R, W - R), :], vsem.at[slot])

    def ocp(i):
        rows = pl.ds(WO_OFFS[i], WO_CHUNKS[i])
        return pltpu.make_async_copy(wo_hbm.at[rows, :], wo_v.at[rows, :], osem.at[i])

    def a_v(h, j):
        s = (2 * h + j) % NS
        return pltpu.make_async_copy(v_hbm.at[0, h, pl.ds(SK - W + j * SV, SV), :], stg_v.at[s], asem.at[s])

    def b_v(h, j):
        s = (2 * h + j) % NS
        return pltpu.make_async_copy(stg_v.at[s], vbuf.at[h % NB, pl.ds(j * SV, SV), :], bsem.at[s])

    def a_o(p):
        s = (p + NS - NPRE) % NS
        return pltpu.make_async_copy(wo_hbm.at[pl.ds(p * SO, SO), :], stg_o.at[s], asem.at[s])

    def b_o(p):
        s = (p + NS - NPRE) % NS
        return pltpu.make_async_copy(stg_o.at[s], wo_v.at[pl.ds(p * SO, SO), :], bsem.at[s])

    def a_e(e):
        return a_o(e + NPRE) if e < 0 else (a_v(e // 2, e % 2) if e < 2 * H else a_o(e - 2 * H + NPRE))

    def b_e(e):
        return b_o(e + NPRE) if e < 0 else (b_v(e // 2, e % 2) if e < 2 * H else b_o(e - 2 * H + NPRE))

    def side_static(k):
        lo, hi = -NPRE, 2 * H + NPOST
        if lo <= k + 2 < hi:
            b_e(k + 2).wait()
        if lo <= k + 6 < hi:
            a_e(k + 6).start()
        if lo <= k + 4 < hi:
            a_e(k + 4).wait()
            b_e(k + 4).start()

    def side_step(h, j):
        @pl.when(h + 1 < H)
        def _():
            b_v(h + 1, j).wait()

        @pl.when(h + 1 >= H)
        def _():
            b_o(NPRE + 2 * (h + 1 - H) + j).wait()

        @pl.when(h + 3 < H)
        def _():
            a_v(h + 3, j).start()

        @pl.when(h + 3 >= H)
        def _():
            a_o(NPRE + 2 * (h + 3 - H) + j).start()

        @pl.when(h + 2 < H)
        def _():
            a_v(h + 2, j).wait()
            b_v(h + 2, j).start()

        @pl.when(h + 2 >= H)
        def _():
            p = NPRE + 2 * (h + 2 - H) + j
            a_o(p).wait()
            b_o(p).start()

    cx.start()
    for i in range(QC):
        qcp(i).start()
    c3.start()
    c4.start()
    side_static(-8)
    side_static(-7)

    cx.wait()
    x8 = jnp.broadcast_to(x_v[0].astype(f32), (8, D))
    xn8 = _ln(x8)
    y8 = _ln(xn8).astype(bf16)
    for i in range(QC):
        qcp(i).wait()
        if i < LA:
            kcp(i, i).start()
            vcp(i, i).start()
        side_static(-6 + i)
    q = jnp.dot(xn8.astype(bf16), wq_v[...], preferred_element_type=f32).astype(bf16)
    for h in range(H):
        q_s[h] = q[:, h * DH:(h + 1) * DH]
    c3.wait()
    side_static(-2)
    h1 = jax.lax.dot_general(y8, w3_v[...], (((1,), (1,)), ((), ())), preferred_element_type=f32)
    h1 = jax.nn.gelu(h1, approximate=True).astype(bf16)
    c4.wait()
    side_static(-1)
    b = xn8 + jnp.dot(h1, w4_v[...], preferred_element_type=f32)
    g = b * jax.nn.sigmoid(b)

    def head(h, carry):
        slot = h % NB
        nslot = (h + LA) % NB
        kcp(h, slot).wait()

        @pl.when(h + LA < H)
        def _():
            kcp(h + LA, nslot).start()

        side_step(h, 0)

        s = jax.lax.dot_general(q_s[h], kbuf[slot], (((1,), (1,)), ((), ())),
                                preferred_element_type=f32) * (DH ** -0.5)
        m = jnp.max(s, axis=-1, keepdims=True)
        p = jnp.exp(s - m)
        l = jnp.sum(p, axis=-1, keepdims=True)
        pb = p.astype(bf16)
        vcp(h, slot).wait()

        @pl.when(h + LA < H)
        def _():
            vcp(h + LA, nslot).start()

        @pl.when(h == H - LA)
        def _():
            for i in range(len(WO_CHUNKS)):
                ocp(i).start()

        side_step(h, 1)

        o = jnp.dot(pb, vbuf[slot], preferred_element_type=f32) / l
        o_s[h] = o.astype(bf16)
        return carry

    jax.lax.fori_loop(0, H, head, 0)

    o_last = o_s[H - 1].astype(f32)
    ob = jnp.transpose(jnp.broadcast_to(o_last[0:1], (DH, DH)))

    def mxu_rows(r0, n):
        h0, nh = r0 // DH, n // DH
        oc = jnp.concatenate([o_s[h0 + j] for j in range(nh)], axis=-1) if nh > 1 else o_s[h0]
        return jnp.dot(oc, wo_v[pl.ds(r0, n), :], preferred_element_type=f32)

    acc = jnp.zeros((8, D), f32)
    nm = len(MXU_CHUNKS)
    for i in range(nm):
        ocp(i).wait()
        if i < 2:
            side_static(2 * H + i)
        if i == 2:
            side_static(2 * H + 2)
            side_static(2 * H + 3)
            acc = acc + mxu_rows(0, RO)
        acc = acc + mxu_rows(WO_OFFS[i], MXU_CHUNKS[i])

    def vpu_rows(i):
        n = WO_CHUNKS[i]
        r0 = WO_OFFS[i] - (H - 1) * DH
        w = wo_v[pl.ds(WO_OFFS[i], n), :].astype(f32)
        prod = w * jnp.concatenate([ob[r0:r0 + n, :]] * (D // DH), axis=1)
        parts = [prod[8 * j:8 * j + 8] for j in range(n // 8)]
        while len(parts) > 1:
            parts = [parts[j] + parts[j + 1] if j + 1 < len(parts) else parts[j]
                     for j in range(0, len(parts), 2)]
        return jnp.sum(parts[0], axis=0, keepdims=True)

    n_all = len(WO_CHUNKS)
    for i in range(nm, n_all - 1):
        ocp(i).wait()
        acc = acc + vpu_rows(i)
    base = x8 + acc * g
    ocp(n_all - 1).wait()
    out = base + vpu_rows(n_all - 1) * g
    out_v[0] = out[0:1].astype(bf16)
    co = pltpu.make_async_copy(out_v, o_hbm, wsem.at[0])
    co.start()
    co.wait()


@jax.jit
def pallas_recurrent_scan__sliding_block_cached__mixer_s_mlp__decode_kernel(
    A_x, A_k_cache, A_v_cache, A_wq, A_wo, B_x, B_w1, B_w2, B_w3, B_w4):
    return pl.pallas_call(
        _kernel,
        in_specs=[pl.BlockSpec(memory_space=pl.ANY)] * 7,
        out_specs=pl.BlockSpec(memory_space=pl.ANY),
        out_shape=jax.ShapeDtypeStruct((1, 1, D), bf16),
        scratch_shapes=[
            pltpu.VMEM((1, 1, D), bf16),
            pltpu.VMEM((D, H * DH), bf16),
            pltpu.VMEM((H * DH, D), bf16),
            pltpu.VMEM((F, D), bf16),
            pltpu.VMEM((F, D), bf16),
            pltpu.VMEM((NB, W, DH), bf16),
            pltpu.VMEM((NB, W, DH), bf16),
            pltpu.VMEM((H, 8, DH), bf16),
            pltpu.VMEM((H, 8, DH), bf16),
            pltpu.VMEM((1, 1, D), bf16),
            pltpu.SMEM((NS, SV, DH), bf16),
            pltpu.SMEM((NS, SO, D), bf16),
            pltpu.SemaphoreType.DMA((3 + QC,)),
            pltpu.SemaphoreType.DMA((NB,)),
            pltpu.SemaphoreType.DMA((NB,)),
            pltpu.SemaphoreType.DMA((len(WO_CHUNKS),)),
            pltpu.SemaphoreType.DMA((NS,)),
            pltpu.SemaphoreType.DMA((NS,)),
        ],
        compiler_params=pltpu.CompilerParams(
            vmem_limit_bytes=64 * 1024 * 1024,
            disable_bounds_checks=True,
            disable_semaphore_checks=True,
        ),
    )(A_x, A_k_cache, A_v_cache, A_wq, A_wo, B_w3.T, B_w4)
```

```python
import jax
import jax.numpy as jnp
import jax.experimental.pallas as pl
import jax.experimental.pallas.tpu as pltpu

H, DH, D, F, W, SK = 32, 128, 512, 1376, 4096, 32768
LA = 2
NB = LA + 1
f32, bf16 = jnp.float32, jnp.bfloat16

S0, S1 = 128, 128
SIDE = (S0, S1)
SV = max(SIDE)
R = S0 + S1
SO = 32
NPRE = 0
NPOST = 6
FP = 32
NF = F // FP
FPI = 3
HSW = -(-NF // FPI)
assert 2 * HSW <= H - LA
F0, F1 = (0, 1), (2,)
RO = (NPRE + NPOST) * SO
NS = 4
QC = 4

MXU_CHUNKS = (1024 - RO, 1024, 1024, 512, 256, 128)
VPU_CHUNKS = (96, 32)
WO_CHUNKS = MXU_CHUNKS + VPU_CHUNKS
WO_OFFS = tuple(RO + sum(WO_CHUNKS[:i]) for i in range(len(WO_CHUNKS)))
assert RO + sum(WO_CHUNKS) == H * DH and sum(VPU_CHUNKS) == DH and F % FP == 0


def _ln(x):
    m = jnp.mean(x, axis=-1, keepdims=True)
    xc = x - m
    v = jnp.mean(xc * xc, axis=-1, keepdims=True)
    return xc / jnp.sqrt(v + 1e-5)


def _kernel(x_hbm, k_hbm, v_hbm, wq_hbm, wo_hbm, w3t_hbm, w4_hbm, o_hbm,
            x_v, wq_v, wo_v, w3_v, w4_v, kbuf, vbuf, q_s, o_s, out_v, stg_v, stg_o,
            wsem, ksem, vsem, osem, asem, bsem, fsem):
    cx = pltpu.make_async_copy(x_hbm, x_v, wsem.at[0])

    def fill_step(h, idxs):
        for i in idxs:
            @pl.when(jnp.logical_and(h < HSW, FPI * h + i < NF))
            def _():
                rows = pl.ds(pl.multiple_of((FPI * h + i) * FP, FP), FP)
                pltpu.make_async_copy(w3t_hbm.at[rows, :], w3_v.at[rows, :], fsem.at[0]).start()

            @pl.when(jnp.logical_and(h >= HSW, FPI * (h - HSW) + i < NF))
            def _():
                rows = pl.ds(pl.multiple_of((FPI * (h - HSW) + i) * FP, FP), FP)
                pltpu.make_async_copy(w4_hbm.at[rows, :], w4_v.at[rows, :], fsem.at[1]).start()

    def qcp(i):
        rows = pl.ds(i * (D // QC), D // QC)
        return pltpu.make_async_copy(wq_hbm.at[rows, :], wq_v.at[rows, :], wsem.at[1 + i])

    def kcp(h, slot):
        return pltpu.make_async_copy(k_hbm.at[0, h, pl.ds(SK - W, W), :], kbuf.at[slot], ksem.at[slot])

    def vcp(h, slot):
        return pltpu.make_async_copy(v_hbm.at[0, h, pl.ds(SK - W + R, W - R), :],
                                     vbuf.at[slot, pl.ds(R, W - R), :], vsem.at[slot])

    def ocp(i):
        rows = pl.ds(WO_OFFS[i], WO_CHUNKS[i])
        return pltpu.make_async_copy(wo_hbm.at[rows, :], wo_v.at[rows, :], osem.at[i])

    def a_v(h, j):
        s = (2 * h + j) % NS
        return pltpu.make_async_copy(v_hbm.at[0, h, pl.ds(SK - W + j * S0, SIDE[j]), :],
                                     stg_v.at[s, pl.ds(0, SIDE[j]), :], asem.at[s])

    def b_v(h, j):
        s = (2 * h + j) % NS
        return pltpu.make_async_copy(stg_v.at[s, pl.ds(0, SIDE[j]), :],
                                     vbuf.at[h % NB, pl.ds(j * S0, SIDE[j]), :], bsem.at[s])

    def a_o(p):
        s = (p + NS - NPRE) % NS
        return pltpu.make_async_copy(wo_hbm.at[pl.ds(p * SO, SO), :], stg_o.at[s], asem.at[s])

    def b_o(p):
        s = (p + NS - NPRE) % NS
        return pltpu.make_async_copy(stg_o.at[s], wo_v.at[pl.ds(p * SO, SO), :], bsem.at[s])

    def a_e(e):
        return a_o(e + NPRE) if e < 0 else (a_v(e // 2, e % 2) if e < 2 * H else a_o(e - 2 * H + NPRE))

    def b_e(e):
        return b_o(e + NPRE) if e < 0 else (b_v(e // 2, e % 2) if e < 2 * H else b_o(e - 2 * H + NPRE))

    def side_static(k):
        lo, hi = -NPRE, 2 * H + NPOST
        if lo <= k + 2 < hi:
            b_e(k + 2).wait()
        if lo <= k + 6 < hi:
            a_e(k + 6).start()
        if lo <= k + 4 < hi:
            a_e(k + 4).wait()
            b_e(k + 4).start()

    def side_step(h, j):
        @pl.when(h + 1 < H)
        def _():
            b_v(h + 1, j).wait()

        @pl.when(jnp.logical_and(h + 1 >= H, 2 * (h + 1 - H) + j < NPOST))
        def _():
            b_o(NPRE + 2 * (h + 1 - H) + j).wait()

        @pl.when(h + 3 < H)
        def _():
            a_v(h + 3, j).start()

        @pl.when(jnp.logical_and(h + 3 >= H, 2 * (h + 3 - H) + j < NPOST))
        def _():
            a_o(NPRE + 2 * (h + 3 - H) + j).start()

        @pl.when(h + 2 < H)
        def _():
            a_v(h + 2, j).wait()
            b_v(h + 2, j).start()

        @pl.when(jnp.logical_and(h + 2 >= H, 2 * (h + 2 - H) + j < NPOST))
        def _():
            p = NPRE + 2 * (h + 2 - H) + j
            a_o(p).wait()
            b_o(p).start()

    cx.start()
    for i in range(QC):
        qcp(i).start()
    for h in range(LA):
        kcp(h, h).start()
        vcp(h, h).start()
    side_static(-6)
    side_static(-5)

    cx.wait()
    x8 = jnp.broadcast_to(x_v[0].astype(f32), (8, D))
    xn8 = _ln(x8)
    y8 = _ln(xn8).astype(bf16)
    for i in range(QC):
        qcp(i).wait()
        side_static(-4 + i)
    q = jnp.dot(xn8.astype(bf16), wq_v[...], preferred_element_type=f32).astype(bf16)
    for h in range(H):
        q_s[h] = q[:, h * DH:(h + 1) * DH]

    def head(h, carry):
        slot = h % NB
        nslot = (h + LA) % NB
        kcp(h, slot).wait()

        @pl.when(h + LA < H)
        def _():
            kcp(h + LA, nslot).start()

        side_step(h, 0)
        fill_step(h, F0)

        s = jax.lax.dot_general(q_s[h], kbuf[slot], (((1,), (1,)), ((), ())),
                                preferred_element_type=f32) * (DH ** -0.5)
        m = jnp.max(s, axis=-1, keepdims=True)
        p = jnp.exp(s - m)
        l = jnp.sum(p, axis=-1, keepdims=True)
        pb = p.astype(bf16)
        vcp(h, slot).wait()

        @pl.when(h + LA < H)
        def _():
            vcp(h + LA, nslot).start()

        @pl.when(h == H - LA)
        def _():
            for i in range(len(WO_CHUNKS)):
                ocp(i).start()

        side_step(h, 1)
        fill_step(h, F1)

        o = jnp.dot(pb, vbuf[slot], preferred_element_type=f32) / l
        o_s[h] = o.astype(bf16)
        return carry

    jax.lax.fori_loop(0, H, head, 0)

    pltpu.make_async_copy(w3_v, w3_v, fsem.at[0]).wait()
    h1 = jax.lax.dot_general(y8, w3_v[...], (((1,), (1,)), ((), ())), preferred_element_type=f32)
    h1 = jax.nn.gelu(h1, approximate=True).astype(bf16)
    pltpu.make_async_copy(w4_v, w4_v, fsem.at[1]).wait()
    b = xn8 + jnp.dot(h1, w4_v[...], preferred_element_type=f32)
    g = b * jax.nn.sigmoid(b)

    o_last = o_s[H - 1].astype(f32)
    ob = jnp.transpose(jnp.broadcast_to(o_last[0:1], (DH, DH)))

    def mxu_rows(r0, n):
        h0, h1_ = r0 // DH, (r0 + n + DH - 1) // DH
        oc = jnp.concatenate([o_s[j] for j in range(h0, h1_)], axis=-1) if h1_ - h0 > 1 else o_s[h0]
        if r0 % DH or n % DH:
            oc = oc[:, r0 - h0 * DH:r0 - h0 * DH + n]
        return jnp.dot(oc, wo_v[pl.ds(r0, n), :], preferred_element_type=f32)

    acc = jnp.zeros((8, D), f32)
    nm = len(MXU_CHUNKS)
    for i in range(nm):
        ocp(i).wait()
        if i < 2:
            side_static(2 * H + i)
        if i == 2:
            side_static(2 * H + 2)
            side_static(2 * H + 3)
            if RO:
                acc = acc + mxu_rows(0, RO)
        acc = acc + mxu_rows(WO_OFFS[i], MXU_CHUNKS[i])

    def vpu_rows(i):
        n = WO_CHUNKS[i]
        r0 = WO_OFFS[i] - (H - 1) * DH
        w = wo_v[pl.ds(WO_OFFS[i], n), :].astype(f32)
        prod = w * jnp.concatenate([ob[r0:r0 + n, :]] * (D // DH), axis=1)
        parts = [prod[8 * j:8 * j + 8] for j in range(n // 8)]
        while len(parts) > 1:
            parts = [parts[j] + parts[j + 1] if j + 1 < len(parts) else parts[j]
                     for j in range(0, len(parts), 2)]
        return jnp.sum(parts[0], axis=0, keepdims=True)

    n_all = len(WO_CHUNKS)
    for i in range(nm, n_all - 1):
        ocp(i).wait()
        acc = acc + vpu_rows(i)
    base = x8 + acc * g
    ocp(n_all - 1).wait()
    out = base + vpu_rows(n_all - 1) * g
    out_v[0] = out[0:1].astype(bf16)
    co = pltpu.make_async_copy(out_v, o_hbm, wsem.at[0])
    co.start()
    co.wait()


@jax.jit
def pallas_recurrent_scan__sliding_block_cached__mixer_s_mlp__decode_kernel(
    A_x, A_k_cache, A_v_cache, A_wq, A_wo, B_x, B_w1, B_w2, B_w3, B_w4):
    return pl.pallas_call(
        _kernel,
        in_specs=[pl.BlockSpec(memory_space=pl.ANY)] * 7,
        out_specs=pl.BlockSpec(memory_space=pl.ANY),
        out_shape=jax.ShapeDtypeStruct((1, 1, D), bf16),
        scratch_shapes=[
            pltpu.VMEM((1, 1, D), bf16),
            pltpu.VMEM((D, H * DH), bf16),
            pltpu.VMEM((H * DH, D), bf16),
            pltpu.VMEM((F, D), bf16),
            pltpu.VMEM((F, D), bf16),
            pltpu.VMEM((NB, W, DH), bf16),
            pltpu.VMEM((NB, W, DH), bf16),
            pltpu.VMEM((H, 8, DH), bf16),
            pltpu.VMEM((H, 8, DH), bf16),
            pltpu.VMEM((1, 1, D), bf16),
            pltpu.SMEM((NS, SV, DH), bf16),
            pltpu.SMEM((NS, SO, D), bf16),
            pltpu.SemaphoreType.DMA((1 + QC,)),
            pltpu.SemaphoreType.DMA((NB,)),
            pltpu.SemaphoreType.DMA((NB,)),
            pltpu.SemaphoreType.DMA((len(WO_CHUNKS),)),
            pltpu.SemaphoreType.DMA((NS,)),
            pltpu.SemaphoreType.DMA((NS,)),
            pltpu.SemaphoreType.DMA((2,)),
        ],
        compiler_params=pltpu.CompilerParams(
            vmem_limit_bytes=64 * 1024 * 1024,
            disable_bounds_checks=True,
            disable_semaphore_checks=True,
        ),
    )(A_x, A_k_cache, A_v_cache, A_wq, A_wo, B_w3.T, B_w4)
```
